```python
import jax
import jax.numpy as jnp

def _softmax(x, axis=-1):
    return jax.nn.softmax(x, axis=axis)
def _gelu(x):
    return jax.nn.gelu(x, approximate=True)
def _silu(x):
    return jax.nn.silu(x)
def _sigmoid(x):
    return jax.nn.sigmoid(x)
def _layernorm(x, axis=-1, eps=1e-5):
    m = jnp.mean(x, axis=axis, keepdims=True)
    v = jnp.var(x, axis=axis, keepdims=True)
    return (x - m) / jnp.sqrt(v + eps)
def _scatter_add(tgt, idx, src, axis=0):
    return tgt.at[idx].add(src)
def _segment_sum(src, seg, n):
    return jax.ops.segment_sum(src, seg, n)
class _Rng:
    def __init__(self, key):
        self._k = key
    def _next(self):
        self._k, sub = jax.random.split(self._k)
        return sub
    def normal(self, shape):
        return jax.random.normal(self._next(), shape, dtype=jnp.bfloat16)
    def randint(self, lo, hi, shape):
        return jax.random.randint(self._next(), shape, lo, hi, dtype=jnp.int32)
    def uniform(self, shape, lo=0.0, hi=1.0):
        return jax.random.uniform(self._next(), shape, jnp.bfloat16, lo, hi)
    def permutation(self, n):
        return jax.random.permutation(self._next(), n)


kernel_name = 'interleave_layers__sliding_block_cached__dense_activation_gelu__decode'

def _fwd_setup_inputs():
    _rng = _Rng(jax.random.key(int.from_bytes(__import__("os").urandom(4), "little")))
    _w = (lambda a: (lambda t: t.astype(jnp.bfloat16) if jnp.issubdtype(t.dtype, jnp.floating) else t)(jnp.asarray(a)))
    def _A_setup():
        B, Sq, D = 2, 1, 512
        Hq, Hkv, Sk, Dh = 32, 8, 32768, 128
        assert Hq % Hkv == 0, (Hq, Hkv)
        return {
            "x": _w((lambda *s: _rng.normal(s) * 0.05)(B, Sq, D)),
            "k_cache": _w((lambda *s: _rng.normal(s) * 0.05)(B, Hkv, Sk, Dh)),
            "v_cache": _w((lambda *s: _rng.normal(s) * 0.05)(B, Hkv, Sk, Dh)),
            "wq": _w((lambda *s: _rng.normal(s) * 0.05)(D, Hq * Dh) * (D ** -0.5)),
            "wo": _w((lambda *s: _rng.normal(s) * 0.05)(Hq * Dh, D) * ((Hq * Dh) ** -0.5)),
        }
    _A_in = _A_setup()

    def _B_setup():
        B, S, D, F = 2, 1, 512, 1792
        return {
            "x": _w((lambda *s: _rng.normal(s) * 0.05)(B, S, D)),
            "w1": _w((lambda *s: _rng.normal(s) * 0.05)(D, F) * (D ** -0.5)),
            "b1": _w((lambda *s: _rng.normal(s) * 0.05)(F) * 0.01),
            "w2": _w((lambda *s: _rng.normal(s) * 0.05)(F, D) * (F ** -0.5)),
            "b2": _w((lambda *s: _rng.normal(s) * 0.05)(D) * 0.01),
        }
    _B_in = _B_setup()

    return {
        "A_x": _A_in["x"],
        "A_k_cache": _A_in["k_cache"],
        "A_v_cache": _A_in["v_cache"],
        "A_wq": _A_in["wq"],
        "A_wo": _A_in["wo"],
        "B_x": _B_in["x"],
        "B_w1": _B_in["w1"],
        "B_b1": _B_in["b1"],
        "B_w2": _B_in["w2"],
        "B_b2": _B_in["b2"],
    }

def _fwd_reference(A_x, A_k_cache, A_v_cache, A_wq, A_wo, B_x, B_w1, B_b1, B_w2, B_b2):
    def _A_ref(x, k_cache, v_cache, wq, wo):
        B, Sq, D = x.shape
        Hq, Dh = 32, 128
        Hkv, Sk = k_cache.shape[1], k_cache.shape[2]
        W = min(4096, max(256, Sk // 4))
        rep = Hq // Hkv
        q = (lambda x, *d: x.transpose(*d))((x @ wq).reshape(B, Sq, Hq, Dh), 0, 2, 1, 3)
        k = jnp.repeat(k_cache[:, :, Sk - W:, :], rep, axis=1)
        v = jnp.repeat(v_cache[:, :, Sk - W:, :], rep, axis=1)
        scores = jnp.einsum("bhqd,bhkd->bhqk", q, k) * (Dh ** -0.5)
        p = _softmax(scores, axis=-1)
        o = jnp.einsum("bhqk,bhkd->bhqd", p, v)
        return (lambda x, *d: x.transpose(*d))(o, 0, 2, 1, 3).reshape(B, Sq, Hq * Dh) @ wo

    def _B_ref(x, w1, b1, w2, b2):
        h = jnp.einsum("bsd,df->bsf", x, w1) + b1
        h = _gelu(h)
        return jnp.einsum("bsf,fd->bsd", h, w2) + b2

    x = A_x
    x = x + _A_ref(_layernorm(x, axis=-1), A_k_cache, A_v_cache, A_wq, A_wo)
    x = x + _B_ref(_layernorm(x, axis=-1), B_w1, B_b1, B_w2, B_b2)
    x = x + _A_ref(_layernorm(x, axis=-1), A_k_cache, A_v_cache, A_wq, A_wo)
    x = x + _B_ref(_layernorm(x, axis=-1), B_w1, B_b1, B_w2, B_b2)
    return x


def setup_inputs():
    _inp = _fwd_setup_inputs()
    _gk = jax.random.fold_in(jax.random.key(int.from_bytes(__import__("os").urandom(4), "little")), 2**31 - 1)
    _shapes = [[2, 1, 512]]
    _dtypes = ['bfloat16']
    _gks = jax.random.split(_gk, len(_shapes))
    _gs = [jax.random.normal(k, s, dtype=jnp.dtype(d)) * 0.05 for k, s, d in zip(_gks, _shapes, _dtypes)]
    _inp["grad_out"] = _gs[0]
    return _inp

def reference(A_x, A_k_cache, A_v_cache, A_wq, A_wo, B_w1, B_b1, B_w2, B_b2, B_x, grad_out):
    _const = dict(B_x=B_x)
    def _f(*_d):
        return _fwd_reference(**{'A_x': _d[0], 'A_k_cache': _d[1], 'A_v_cache': _d[2], 'A_wq': _d[3], 'A_wo': _d[4], 'B_w1': _d[5], 'B_b1': _d[6], 'B_w2': _d[7], 'B_b2': _d[8], **_const})
    _out, _vjp = jax.vjp(_f, A_x, A_k_cache, A_v_cache, A_wq, A_wo, B_w1, B_b1, B_w2, B_b2)
    _grads = _vjp(grad_out)
    _out0 = jnp.asarray(_out)
    return (_out0, *[jnp.asarray(_g) for _g in _grads])
```

```python
import math

import jax
import jax.numpy as jnp
from jax import lax
import jax.experimental.pallas as pl
import jax.experimental.pallas.tpu as pltpu

HQ = 32
DH = 128
EPS = 1e-5
GELU_C = math.sqrt(2.0 / math.pi)
GELU_A = 0.044715
N_LAYERS = 2
ROWS = 8

ZROWS = 128
RROWS = 32
RHEADS = 4
KCHUNK = 512

F32 = jnp.float32
BF16 = jnp.bfloat16


def _nn(a, b):
  return lax.dot_general(a, b, (((1,), (0,)), ((), ())),
                         preferred_element_type=F32)


def _nt(a, b):
  return lax.dot_general(a, b, (((1,), (1,)), ((), ())),
                         preferred_element_type=F32)


def _tn(a, b):
  return lax.dot_general(a, b, (((0,), (0,)), ((), ())),
                         preferred_element_type=F32)


def _row_iota(shape):
  return lax.broadcasted_iota(jnp.int32, shape, 0)


def _by_batch(v0, v1):
  return jnp.where(_row_iota(v0.shape) % 2 == 0, v0, v1)


def _layernorm(x):
  mean = jnp.mean(x, axis=-1, keepdims=True)
  xc = x - mean
  var = jnp.mean(xc * xc, axis=-1, keepdims=True)
  rstd = 1.0 / jnp.sqrt(var + EPS)
  return xc * rstd, rstd


def _layernorm_bwd(dn, n, rstd):
  return rstd * (dn - jnp.mean(dn, axis=-1, keepdims=True)
                 - n * jnp.mean(dn * n, axis=-1, keepdims=True))


def _sum_head_rows(v):
  v = v + pltpu.roll(v, 4, 0)
  return v + pltpu.roll(v, 2, 0)


def _kernel(x_hbm, k_hbm, v_hbm, wq_hbm, wo_hbm, w1_hbm, b1_hbm, w2_hbm,
            b2_hbm, go_hbm,
            out_hbm, dx_hbm, dk_hbm, dv_hbm, dwq_hbm, dwo_hbm, dw1_hbm,
            db1_hbm, dw2_hbm, db2_hbm,
            xs, gos, b1s, b2s, outs, dxs, db1s, db2s,
            kbuf, vbuf, wq, wo, w1, w2, dwq, dwo, dw1, dw2, zbuf,
            na_s, ra_s, nb_s, rb_s, h_s, g_s, dh_s, da_s, dy_s,
            oe_s, dqe_s, q_s, do_s, hs_s, p_s, ds_s, sel_s,
            rsem, zsem, wsem, ssem):
  nb, hkv, seq, _ = k_hbm.shape
  win = kbuf.shape[2]
  zero_rows = seq - win
  rep = HQ // hkv
  d_ff = w1.shape[1]
  scale = DH ** -0.5
  n_kchunk = win // KCHUNK

  small_in = [pltpu.make_async_copy(s, d, ssem.at[i]) for i, (s, d) in
              enumerate(((x_hbm, xs), (go_hbm, gos), (b1_hbm, b1s),
                         (b2_hbm, b2s)))]

  r_chunks = win // RROWS
  r_groups = hkv // RHEADS

  def read_step(i, carry):
    grp, c = i // r_chunks, i % r_chunks
    b, h0 = grp // r_groups, (grp % r_groups) * RHEADS
    for q, (src, dst) in enumerate(((k_hbm, kbuf), (v_hbm, vbuf))):
      pltpu.make_async_copy(
          src.at[b, pl.ds(h0, RHEADS), pl.ds(zero_rows + c * RROWS, RROWS), :],
          dst.at[b, pl.ds(h0, RHEADS), pl.ds(c * RROWS, RROWS), :],
          rsem.at[q]).start(priority=q)
    return carry

  lax.fori_loop(0, nb * r_groups * r_chunks, read_step, 0)

  for cp in small_in:
    cp.start()
  weights_in = [pltpu.make_async_copy(s, d, rsem.at[2 + i]) for i, (s, d) in
                enumerate(((wq_hbm, wq), (wo_hbm, wo), (w1_hbm, w1),
                           (w2_hbm, w2)))]
  for i, cp in enumerate(weights_in):
    cp.start(priority=i % 2)

  zbuf[...] = jnp.zeros(zbuf.shape, BF16)
  z_chunks = zero_rows // ZROWS
  z_total = nb * z_chunks

  def zero_step(i, carry):
    b, c = i // z_chunks, i % z_chunks
    for q, dst in enumerate((dk_hbm, dv_hbm)):
      pltpu.make_async_copy(
          zbuf, dst.at[b, :, pl.ds(c * ZROWS, ZROWS), :],
          zsem.at[q]).start(priority=q)
    return carry

  def pump(zi, n):
    end = jnp.minimum(zi + n, z_total)
    lax.fori_loop(zi, end, zero_step, 0)
    return end

  zi = pump(jnp.int32(0), 24)

  for cp in small_in:
    cp.wait()
  for q, buf in enumerate((kbuf, vbuf)):
    pltpu.make_async_copy(buf, buf, rsem.at[q]).wait()
  for cp in weights_in:
    cp.wait()

  def replicate(ref):
    v = ref[...].astype(F32)
    shape = (ROWS, v.shape[1])
    return _by_batch(jnp.broadcast_to(v[0:1], shape),
                     jnp.broadcast_to(v[1:2], shape))

  def as_row(ref):
    v = ref[...].astype(F32)
    return jnp.concatenate([v[i:i + 1] for i in range(v.shape[0])], axis=1)

  b1 = as_row(b1s)
  b2 = as_row(b2s)
  head_of_row = _row_iota((ROWS, DH)) // 2

  def to_groups(v, dst, l):
    for g in range(hkv):
      t = v[:, g * rep * DH:(g * rep + 1) * DH]
      for r in range(1, rep):
        h = g * rep + r
        t = jnp.where(head_of_row == r, v[:, h * DH:(h + 1) * DH], t)
      dst[l, g] = t

  def from_groups():
    cols = []
    for g in range(hkv):
      t = hs_s[g]
      cols += [jnp.where(head_of_row == r, t, 0.0) for r in range(rep)]
    return jnp.concatenate(cols, axis=1)

  def put_keys(dst, l, g, v):
    for c in range(n_kchunk):
      dst[c, l * hkv + g] = v[:, c * KCHUNK:(c + 1) * KCHUNK]

  def layer_fwd(l, carry):
    x, zi = carry
    n, rstd = _layernorm(x)
    na_s[l] = n
    ra_s[l] = jnp.broadcast_to(rstd, ra_s.shape[1:])
    to_groups(_nn(n.astype(BF16), wq[...]), q_s, l)

    def group(g, zi):
      zi = pump(zi, 6)
      q = q_s[l, g].astype(BF16)
      s = _by_batch(_nt(q, kbuf[0, g]), _nt(q, kbuf[1, g])) * scale
      e = jnp.exp(s - jnp.max(s, axis=-1, keepdims=True))
      p = e / jnp.sum(e, axis=-1, keepdims=True)
      put_keys(p_s, l, g, p)
      p = p.astype(BF16)
      hs_s[g] = _by_batch(_nn(p, vbuf[0, g]), _nn(p, vbuf[1, g]))
      return zi

    zi = lax.fori_loop(0, hkv, group, zi)
    zi = pump(zi, 12)
    oe = from_groups()
    oe_s[l] = oe
    x = x + _sum_head_rows(_nn(oe.astype(BF16), wo[...]))

    n, rstd = _layernorm(x)
    nb_s[l] = n
    rb_s[l] = jnp.broadcast_to(rstd, rb_s.shape[1:])
    h = _nn(n.astype(BF16), w1[...]) + b1
    h_s[l] = h
    act = 0.5 * h * (1.0 + jnp.tanh(GELU_C * (h + GELU_A * h * h * h)))
    g_s[l] = act
    x = x + _nn(act.astype(BF16), w2[...]) + b2
    return x, zi

  x, zi = lax.fori_loop(0, N_LAYERS, layer_fwd, (replicate(xs), zi))
  outs[...] = x[0:nb].astype(BF16)

  first_copy = _row_iota((ROWS, x.shape[1])) < nb

  def layer_bwd(i, carry):
    dx, zi = carry
    l = N_LAYERS - 1 - i
    dy_s[l] = jnp.where(first_copy, dx, 0.0)
    dact = _nt(dx.astype(BF16), w2[...])
    h = h_s[l]
    t = jnp.tanh(GELU_C * (h + GELU_A * h * h * h))
    dgelu = 0.5 * (1.0 + t) + (0.5 * GELU_C) * h * (1.0 - t * t) * (
        1.0 + (3.0 * GELU_A) * h * h)
    dh = dact * dgelu
    dh_s[l] = jnp.where(_row_iota(dh.shape) < nb, dh, 0.0)
    dn = _nt(dh.astype(BF16), w1[...])
    dx = dx + _layernorm_bwd(dn, nb_s[l], rb_s[l][:, 0:1])

    da_s[l] = dx
    to_groups(_nt(dx.astype(BF16), wo[...]), do_s, l)
    zi = pump(zi, 12)

    def group(g, zi):
      zi = pump(zi, 6)
      do = do_s[l, g].astype(BF16)
      dp = _by_batch(_nt(do, vbuf[0, g]), _nt(do, vbuf[1, g]))
      p = jnp.concatenate(
          [p_s[c, l * hkv + g] for c in range(n_kchunk)], axis=1)
      ds = p * (dp - jnp.sum(p * dp, axis=-1, keepdims=True)) * scale
      put_keys(ds_s, l, g, ds)
      ds = ds.astype(BF16)
      hs_s[g] = _by_batch(_nn(ds, kbuf[0, g]), _nn(ds, kbuf[1, g]))
      return zi

    zi = lax.fori_loop(0, hkv, group, zi)
    dqe = from_groups()
    dqe_s[l] = dqe
    dn = _sum_head_rows(_nt(dqe.astype(BF16), wq[...]))
    dx = dx + _layernorm_bwd(dn, na_s[l], ra_s[l][:, 0:1])
    return dx, zi

  dx, zi = lax.fori_loop(0, N_LAYERS, layer_bwd, (replicate(gos), zi))
  dxs[...] = dx[0:nb].astype(BF16)

  def stacked(ref):
    v = ref[...]
    return v.reshape(v.shape[0] * v.shape[1], v.shape[2])

  zi = pump(zi, 12)
  for dst, act, grad in ((dwq, na_s, dqe_s), (dwo, oe_s, da_s),
                         (dw1, nb_s, dh_s), (dw2, g_s, dy_s)):
    dst[...] = _tn(stacked(act).astype(BF16),
                   stacked(grad).astype(BF16)).astype(BF16)
  for dst, grad in ((db1s, dh_s), (db2s, dy_s)):
    tot = jnp.sum(stacked(grad), axis=0, keepdims=True)
    dst[...] = jnp.concatenate(
        [tot[:, i * 128:(i + 1) * 128] for i in range(dst.shape[0])],
        axis=0).astype(BF16)

  n_rows = N_LAYERS * hkv * ROWS
  row = _row_iota((n_rows, DH))
  owner = (row % 2) * hkv + (row // ROWS) % hkv

  def select_step(j, carry):
    for t, src in enumerate((q_s, do_s)):
      v = src[...].reshape(n_rows, DH)
      sel_s[t, j] = jnp.where(owner == j, v, 0.0).astype(BF16)
    return carry

  lax.fori_loop(0, nb * hkv, select_step, 0)

  def cache_step(c, zi):
    zi = pump(zi, 12)
    keys = pl.ds(pl.multiple_of(c * KCHUNK, KCHUNK), KCHUNK)
    for t, (src, dst) in enumerate(((ds_s, kbuf), (p_s, vbuf))):
      at = src[c].reshape(n_rows, KCHUNK).T.astype(BF16)

      def head_step(j, carry):
        dst[j // hkv, j % hkv, keys, :] = _nn(at, sel_s[t, j]).astype(BF16)
        return carry

      lax.fori_loop(0, nb * hkv, head_step, 0)
    return zi

  zi = lax.fori_loop(0, n_kchunk, cache_step, zi)

  small_out = [pltpu.make_async_copy(s, d, ssem.at[i]) for i, (s, d) in
               enumerate(((outs, out_hbm), (dxs, dx_hbm), (db1s, db1_hbm),
                          (db2s, db2_hbm)))]
  for cp in small_out:
    cp.start()
  weights_out = [pltpu.make_async_copy(s, d, wsem.at[2 + i]) for i, (s, d) in
                 enumerate(((dwq, dwq_hbm), (dwo, dwo_hbm), (dw1, dw1_hbm),
                            (dw2, dw2_hbm)))]
  for i, cp in enumerate(weights_out):
    cp.start(priority=i % 2)

  pump(zi, z_total)

  w_chunks = win // ZROWS

  def window_step(i, carry):
    b, c = i // w_chunks, i % w_chunks
    for q, (src, dst) in enumerate(((kbuf, dk_hbm), (vbuf, dv_hbm))):
      pltpu.make_async_copy(
          src.at[b, :, pl.ds(c * ZROWS, ZROWS), :],
          dst.at[b, :, pl.ds(zero_rows + c * ZROWS, ZROWS), :],
          wsem.at[q]).start(priority=q)
    return carry

  lax.fori_loop(0, nb * w_chunks, window_step, 0)

  for cp in small_out + weights_out:
    cp.wait()
  for q, (buf, dst) in enumerate(((kbuf, dk_hbm), (vbuf, dv_hbm))):
    zeros = dst.at[:, :, pl.ds(0, zero_rows), :]
    pltpu.make_async_copy(zeros, zeros, zsem.at[q]).wait()
    pltpu.make_async_copy(buf, buf, wsem.at[q]).wait()


@jax.jit
def pallas_interleave_layers__sliding_block_cached__dense_activation_gelu__decode_kernel(
    A_x: jax.Array,
    A_k_cache: jax.Array,
    A_v_cache: jax.Array,
    A_wq: jax.Array,
    A_wo: jax.Array,
    B_x: jax.Array,
    B_w1: jax.Array,
    B_b1: jax.Array,
    B_w2: jax.Array,
    B_b2: jax.Array,
    grad_out: jax.Array,
):
  del B_x
  nb, sq, d = A_x.shape
  _, hkv, seq, dh = A_k_cache.shape
  d_ff = B_w1.shape[1]
  win = min(4096, max(256, seq // 4))
  assert (nb, sq, dh, HQ // hkv) == (2, 1, DH, 4)
  assert win % KCHUNK == 0 and win % ZROWS == 0 and win % RROWS == 0
  assert (seq - win) % ZROWS == 0 and hkv % RHEADS == 0
  assert d % 128 == 0 and d_ff % 128 == 0

  row2 = (nb, d)
  b1_shape = (d_ff // 128, 128)
  b2_shape = (d // 128, 128)
  inputs = (A_x.reshape(row2), A_k_cache, A_v_cache, A_wq, A_wo, B_w1,
            B_b1.reshape(b1_shape), B_w2, B_b2.reshape(b2_shape),
            grad_out.reshape(row2))
  out_shapes = (row2, row2, A_k_cache.shape, A_v_cache.shape, A_wq.shape,
                A_wo.shape, B_w1.shape, b1_shape, B_w2.shape, b2_shape)

  def act(n):
    return pltpu.VMEM((N_LAYERS, ROWS, n), F32)

  weights = [pltpu.VMEM(w.shape, BF16) for w in (A_wq, A_wo, B_w1, B_w2)]
  n_kchunk = win // KCHUNK
  scratch = [
      *[pltpu.VMEM(s, BF16) for s in (row2, row2, b1_shape, b2_shape)] * 2,
      *[pltpu.VMEM((nb, hkv, win, dh), BF16)] * 2,
      *weights, *weights,
      pltpu.VMEM((hkv, ZROWS, dh), BF16),
      act(d), act(128), act(d), act(128), act(d_ff), act(d_ff), act(d_ff),
      act(d), act(d), act(HQ * DH), act(HQ * DH),
      *[pltpu.VMEM((N_LAYERS, hkv, ROWS, DH), F32)] * 2,
      pltpu.VMEM((hkv, ROWS, DH), F32),
      *[pltpu.VMEM((n_kchunk, N_LAYERS * hkv, ROWS, KCHUNK), F32)] * 2,
      pltpu.VMEM((2, nb * hkv, N_LAYERS * hkv * ROWS, DH), BF16),
      pltpu.SemaphoreType.DMA((6,)),
      pltpu.SemaphoreType.DMA((2,)),
      pltpu.SemaphoreType.DMA((6,)),
      pltpu.SemaphoreType.DMA((4,)),
  ]

  outs = pl.pallas_call(
      _kernel,
      out_shape=[jax.ShapeDtypeStruct(s, BF16) for s in out_shapes],
      in_specs=[pl.BlockSpec(memory_space=pltpu.HBM)] * len(inputs),
      out_specs=[pl.BlockSpec(memory_space=pltpu.HBM)] * len(out_shapes),
      scratch_shapes=scratch,
      compiler_params=pltpu.CompilerParams(
          vmem_limit_bytes=100 * 1024 * 1024),
  )(*inputs)
  out, dx, dk, dv, dwq, dwo, dw1, db1, dw2, db2 = outs
  return (out.reshape(A_x.shape), dx.reshape(A_x.shape), dk, dv, dwq, dwo,
          dw1, db1.reshape(B_b1.shape), dw2, db2.reshape(B_b2.shape))
```

```python
import math

import jax
import jax.numpy as jnp
from jax import lax
import jax.experimental.pallas as pl
import jax.experimental.pallas.tpu as pltpu

HQ = 32
DH = 128
EPS = 1e-5
GELU_C = math.sqrt(2.0 / math.pi)
GELU_A = 0.044715
N_LAYERS = 2
ROWS = 8

ZROWS = 112
ZHEADS = 4
OROWS = 32
WSEG = 4
WPOS = "mid"
EARLY = 0
RROWS = 32
RHEADS = 4
KCHUNK = 512
FCHUNK = 256
PUMP0 = 32
PUMP_G = 12
PUMP_F = 3
PUMP_W = 6
PUMP_C = 32
ZW = True
NOBC = False

F32 = jnp.float32
BF16 = jnp.bfloat16


def _nn(a, b):
  return lax.dot_general(a, b, (((1,), (0,)), ((), ())),
                         preferred_element_type=F32)


def _nt(a, b):
  return lax.dot_general(a, b, (((1,), (1,)), ((), ())),
                         preferred_element_type=F32)


def _tn(a, b):
  return lax.dot_general(a, b, (((0,), (0,)), ((), ())),
                         preferred_element_type=F32)


def _row_iota(shape):
  return lax.broadcasted_iota(jnp.int32, shape, 0)


def _by_batch(v0, v1):
  return jnp.where(_row_iota(v0.shape) % 2 == 0, v0, v1)


def _layernorm(x):
  mean = jnp.mean(x, axis=-1, keepdims=True)
  xc = x - mean
  var = jnp.mean(xc * xc, axis=-1, keepdims=True)
  rstd = 1.0 / jnp.sqrt(var + EPS)
  return xc * rstd, rstd


def _layernorm_bwd(dn, n, rstd):
  return rstd * (dn - jnp.mean(dn, axis=-1, keepdims=True)
                 - n * jnp.mean(dn * n, axis=-1, keepdims=True))


def _sum_head_rows(v):
  v = v + pltpu.roll(v, 4, 0)
  return v + pltpu.roll(v, 2, 0)


def _chunk(i, size):
  return pl.ds(pl.multiple_of(i * size, size), size)


def _loop(lo, hi, body):
  lax.fori_loop(lo, hi, lambda i, c: (body(i), c)[1], 0)


def _kernel(x_hbm, k_hbm, v_hbm, wq_hbm, wo_hbm, w1_hbm, b1_hbm, w2_hbm,
            b2_hbm, go_hbm,
            out_hbm, dx_hbm, dk_hbm, dv_hbm, dwq_hbm, dwo_hbm, dw1_hbm,
            db1_hbm, dw2_hbm, db2_hbm,
            xs, gos, b1s, b2s, outs, dxs, db1s, db2s,
            kbuf, vbuf, wq, wo, w1, w2, dwq, dwo, dw1, dw2, zbuf,
            na_s, ra_s, nb_s, rb_s, h_s, g_s, dh_s, da_s, dy_s,
            oe_s, dqe_s, q_s, do_s, b1_s, p_s, ds_s, sel_s,
            rsem, zsem, wsem, ssem):
  nb, hkv, seq, _ = k_hbm.shape
  win = kbuf.shape[2]
  zero_rows = seq - win
  rep = HQ // hkv
  gw = rep * DH
  d_model, d_ff = w1.shape
  scale = DH ** -0.5
  n_kchunk = win // KCHUNK
  n_fchunk = d_ff // FCHUNK

  r_chunks = win // RROWS
  r_groups = hkv // RHEADS

  def read_step(i):
    grp, c = i // r_chunks, i % r_chunks
    b, h0 = grp // r_groups, (grp % r_groups) * RHEADS
    for q, (src, dst) in enumerate(((k_hbm, kbuf), (v_hbm, vbuf))):
      pltpu.make_async_copy(
          src.at[b, pl.ds(h0, RHEADS), pl.ds(zero_rows + c * RROWS, RROWS), :],
          dst.at[b, pl.ds(h0, RHEADS), pl.ds(c * RROWS, RROWS), :],
          rsem.at[q]).start(priority=q)

  _loop(0, nb * r_groups * r_chunks, read_step)

  w_hbm = (wq_hbm, wo_hbm, w1_hbm, w2_hbm)
  w_vmem = (wq, wo, w1, w2)
  dw_hbm = (dwq_hbm, dwo_hbm, dw1_hbm, dw2_hbm)
  dw_vmem = (dwq, dwo, dw1, dw2)

  def move_weights(src, dst, sem, nseg):
    src, dst = ([r.reshape(nseg, r.shape[0] // nseg, r.shape[1]) for r in refs]
                for refs in (src, dst))

    def start(t, rows, cols):
      pltpu.make_async_copy(src[t].at[:, rows, cols], dst[t].at[:, rows, cols],
                            sem.at[2 + t]).start(priority=t % 2)

    for up, down, width in ((0, 1, 1024), (2, 3, 896)):
      per_band = src[up].shape[2] // width
      n_up = src[up].shape[1] // 16 * per_band
      n_down = src[down].shape[1] // 32

      def step(i):
        start(up, pl.ds(i // per_band * 16, 16),
              pl.ds(i % per_band * width, width))
        if n_down == n_up:
          start(down, pl.ds(i * 32, 32), slice(None))
        else:
          pl.when(i < n_down)(
              lambda: start(down, pl.ds(i * 32, 32), slice(None)))

      _loop(0, n_up, step)

  move_weights(w_hbm, w_vmem, rsem, 1)

  small_in = [pltpu.make_async_copy(s, d, ssem.at[i]) for i, (s, d) in
              enumerate(((x_hbm, xs), (go_hbm, gos), (b1_hbm, b1s),
                         (b2_hbm, b2s)))]
  for cp in small_in:
    cp.start()

  zbuf[...] = jnp.zeros(zbuf.shape, BF16)
  z_chunks = zero_rows // ZROWS
  z_groups = hkv // ZHEADS
  z_total = nb * z_groups * z_chunks

  def zero_step(i):
    if not ZW: return
    grp, c = i // z_chunks, i % z_chunks
    b, h0 = grp // z_groups, (grp % z_groups) * ZHEADS
    for q, dst in enumerate((dk_hbm, dv_hbm)):
      pltpu.make_async_copy(
          zbuf, dst.at[b, pl.ds(h0, ZHEADS), pl.ds(c * ZROWS, ZROWS), :],
          zsem.at[q]).start(priority=q)

  def pump(zi, n):
    _loop(zi, zi + n, zero_step)
    return zi + n

  zi = pump(jnp.int32(0), PUMP0)
  z_planned = (PUMP0 + 2 * N_LAYERS * (hkv * PUMP_G + n_fchunk * PUMP_F)
               + (hkv + n_fchunk) * PUMP_W)
  assert z_planned + n_kchunk * PUMP_C <= z_total

  for cp in small_in:
    cp.wait()
  for q, buf in enumerate((kbuf, vbuf) + w_vmem):
    pltpu.make_async_copy(buf, buf, rsem.at[q]).wait()

  def replicate(ref):
    v = ref[...].astype(F32)
    shape = (ROWS, v.shape[1])
    return _by_batch(jnp.broadcast_to(v[0:1], shape),
                     jnp.broadcast_to(v[1:2], shape))

  def as_rows(ref):
    v = ref[...].astype(F32)
    return jnp.concatenate(
        [jnp.broadcast_to(v[i:i + 1], (ROWS, 128)) for i in range(v.shape[0])],
        axis=1)

  b1_s[...] = as_rows(b1s)
  b2 = as_rows(b2s)
  head_of_row = _row_iota((ROWS, DH)) // 2

  def gather_heads(v):
    t = v[:, 0:DH]
    for r in range(1, rep):
      t = jnp.where(head_of_row == r, v[:, r * DH:(r + 1) * DH], t)
    return t

  def scatter_heads(t):
    return jnp.concatenate(
        [jnp.where(head_of_row == r, t, 0.0) for r in range(rep)], axis=1)

  def keys_row(l, g):
    return pl.ds(pl.multiple_of((l * hkv + g) * ROWS, ROWS), ROWS)

  def layer_row(l):
    return pl.ds(pl.multiple_of(l * ROWS, ROWS), ROWS)

  def layer_fwd(l, carry):
    x, zi = carry
    rows = layer_row(l)
    n, rstd = _layernorm(x)
    na_s[rows, :] = n
    ra_s[rows, :] = jnp.broadcast_to(rstd, (ROWS, 128))
    n = n.astype(BF16)

    def group(g, carry):
      acc, zi = carry
      zi = pump(zi, PUMP_G)
      cols = _chunk(g, gw)
      q = gather_heads(_nn(n, wq[:, cols]))
      q_s[keys_row(l, g), :] = q
      q = q.astype(BF16)
      s = _by_batch(_nt(q, kbuf[0, g]), _nt(q, kbuf[1, g])) * scale
      e = jnp.exp(s - jnp.max(s, axis=-1, keepdims=True))
      p = e / jnp.sum(e, axis=-1, keepdims=True)
      p_s[keys_row(l, g), :] = p
      p = p.astype(BF16)
      oe = scatter_heads(
          _by_batch(_nn(p, vbuf[0, g]), _nn(p, vbuf[1, g])))
      oe_s[rows, cols] = oe
      return acc + _nn(oe.astype(BF16), wo[cols, :]), zi

    acc, zi = lax.fori_loop(0, hkv, group, (jnp.zeros_like(x), zi))
    x = x + _sum_head_rows(acc)

    n2, rstd = _layernorm(x)
    nb_s[rows, :] = n2
    rb_s[rows, :] = jnp.broadcast_to(rstd, (ROWS, 128))
    n2 = n2.astype(BF16)

    def hidden(j, carry):
      acc, zi = carry
      zi = pump(zi, PUMP_F)
      cols = _chunk(j, FCHUNK)
      h = _nn(n2, w1[:, cols]) + b1_s[:, cols]
      h_s[rows, cols] = h
      act = 0.5 * h * (1.0 + jnp.tanh(GELU_C * (h + GELU_A * h * h * h)))
      g_s[rows, cols] = act
      return acc + _nn(act.astype(BF16), w2[cols, :]), zi

    acc, zi = lax.fori_loop(0, n_fchunk, hidden, (b2, zi))
    return x + acc, zi

  x, zi = lax.fori_loop(0, N_LAYERS, layer_fwd, (replicate(xs), zi))
  outs[...] = x[0:nb].astype(BF16)

  def first_copy(v):
    return jnp.where(_row_iota(v.shape) < nb, v, 0.0)

  def layer_bwd(i, carry):
    dx, zi = carry
    l = N_LAYERS - 1 - i
    rows = layer_row(l)
    dy_s[rows, :] = first_copy(dx)
    dy = dx.astype(BF16)

    def hidden(j, carry):
      acc, zi = carry
      zi = pump(zi, PUMP_F)
      cols = _chunk(j, FCHUNK)
      h = h_s[rows, cols]
      t = jnp.tanh(GELU_C * (h + GELU_A * h * h * h))
      dgelu = 0.5 * (1.0 + t) + (0.5 * GELU_C) * h * (1.0 - t * t) * (
          1.0 + (3.0 * GELU_A) * h * h)
      dh = _nt(dy, w2[cols, :]) * dgelu
      dh_s[rows, cols] = first_copy(dh)
      return acc + _nt(dh.astype(BF16), w1[:, cols]), zi

    dn, zi = lax.fori_loop(0, n_fchunk, hidden, (jnp.zeros_like(dx), zi))
    dx = dx + _layernorm_bwd(dn, nb_s[rows, :], rb_s[rows, 0:1])
    da_s[rows, :] = dx
    da = dx.astype(BF16)

    def group(g, carry):
      acc, zi = carry
      zi = pump(zi, PUMP_G)
      cols = _chunk(g, gw)
      do = gather_heads(_nt(da, wo[cols, :]))
      do_s[keys_row(l, g), :] = do
      do = do.astype(BF16)
      dp = _by_batch(_nt(do, vbuf[0, g]), _nt(do, vbuf[1, g]))
      p = p_s[keys_row(l, g), :]
      ds = p * (dp - jnp.sum(p * dp, axis=-1, keepdims=True)) * scale
      ds_s[keys_row(l, g), :] = ds
      ds = ds.astype(BF16)
      dqe = scatter_heads(
          _by_batch(_nn(ds, kbuf[0, g]), _nn(ds, kbuf[1, g])))
      dqe_s[rows, cols] = dqe
      return acc + _nt(dqe.astype(BF16), wq[:, cols]), zi

    dn, zi = lax.fori_loop(0, hkv, group, (jnp.zeros_like(dx), zi))
    dx = dx + _layernorm_bwd(_sum_head_rows(dn), na_s[rows, :],
                             ra_s[rows, 0:1])
    return dx, zi

  dx, zi = lax.fori_loop(0, N_LAYERS, layer_bwd, (replicate(gos), zi))
  dxs[...] = dx[0:nb].astype(BF16)

  def weight_grads(n, size, up_act, up_grad, up, down_act, down_grad, down, zi):
    a = up_act[...].T.astype(BF16)
    dg = down_grad[...].astype(BF16)

    def step(j, zi):
      zi = pump(zi, PUMP_W)
      cols = _chunk(j, size)
      up[:, cols] = _nn(a, up_grad[:, cols].astype(BF16)).astype(BF16)
      down[cols, :] = _nn(down_act[:, cols].T.astype(BF16), dg).astype(BF16)
      return zi

    return lax.fori_loop(0, n, step, zi)

  zi = weight_grads(hkv, gw, na_s, dqe_s, dwq, oe_s, da_s, dwo, zi)
  zi = weight_grads(n_fchunk, FCHUNK, nb_s, dh_s, dw1, g_s, dy_s, dw2, zi)
  for dst, grad in ((db1s, dh_s), (db2s, dy_s)):
    tot = jnp.sum(grad[...], axis=0, keepdims=True)
    dst[...] = jnp.concatenate(
        [tot[:, i * 128:(i + 1) * 128] for i in range(dst.shape[0])],
        axis=0).astype(BF16)

  small_out = [pltpu.make_async_copy(s, d, ssem.at[i]) for i, (s, d) in
               enumerate(((outs, out_hbm), (dxs, dx_hbm), (db1s, db1_hbm),
                          (db2s, db2_hbm)))]
  for cp in small_out:
    cp.start()

  if WPOS == "mid":
    move_weights(dw_vmem, dw_hbm, wsem, WSEG)

  n_rows = N_LAYERS * hkv * ROWS
  row = _row_iota((n_rows, DH))
  owner = (row % 2) * hkv + (row // ROWS) % hkv

  def select_step(j):
    for t, src in enumerate((q_s, do_s)):
      sel_s[t, j] = jnp.where(owner == j, src[...], 0.0).astype(BF16)

  _loop(0, nb * hkv, select_step)

  def cache_step(c):
    pump(z_planned + c * PUMP_C, PUMP_C)
    keys = _chunk(c, KCHUNK)
    for t, (src, dst) in enumerate(((ds_s, kbuf), (p_s, vbuf))):
      at = src[:, keys].T.astype(BF16)

      def head_step(j):
        dst[j // hkv, j % hkv, keys, :] = _nn(at, sel_s[t, j]).astype(BF16)

      _loop(0, nb * hkv, head_step)

  _loop(0, n_kchunk, cache_step)

  _loop(z_planned + n_kchunk * PUMP_C, z_total, zero_step)
  if WPOS == "end":
    move_weights(dw_vmem, dw_hbm, wsem, WSEG)

  o_chunks = win // OROWS

  def window_step(i):
    grp, c = i // o_chunks, i % o_chunks
    b, h0 = grp // z_groups, (grp % z_groups) * ZHEADS
    for q, (src, dst) in enumerate(((kbuf, dk_hbm), (vbuf, dv_hbm))):
      pltpu.make_async_copy(
          src.at[b, pl.ds(h0, ZHEADS), pl.ds(c * OROWS, OROWS), :],
          dst.at[b, pl.ds(h0, ZHEADS), pl.ds(zero_rows + c * OROWS, OROWS), :],
          wsem.at[q]).start(priority=q)

  _loop(0, nb * z_groups * o_chunks, window_step)

  for cp in small_out:
    cp.wait()
  for q, buf in enumerate((kbuf, vbuf) + dw_vmem):
    pltpu.make_async_copy(buf, buf, wsem.at[q]).wait()
  for q, dst in enumerate((dk_hbm, dv_hbm)):
    zeros = dst.at[:, :, pl.ds(0, zero_rows), :]
    if ZW: pltpu.make_async_copy(zeros, zeros, zsem.at[q]).wait()


@jax.jit
def pallas_interleave_layers__sliding_block_cached__dense_activation_gelu__decode_kernel(
    A_x: jax.Array,
    A_k_cache: jax.Array,
    A_v_cache: jax.Array,
    A_wq: jax.Array,
    A_wo: jax.Array,
    B_x: jax.Array,
    B_w1: jax.Array,
    B_b1: jax.Array,
    B_w2: jax.Array,
    B_b2: jax.Array,
    grad_out: jax.Array,
):
  del B_x
  nb, sq, d = A_x.shape
  _, hkv, seq, dh = A_k_cache.shape
  d_ff = B_w1.shape[1]
  win = min(4096, max(256, seq // 4))
  assert (nb, sq, dh, HQ // hkv) == (2, 1, DH, 4)
  assert win % KCHUNK == 0 and win % OROWS == 0 and win % RROWS == 0
  assert (seq - win) % ZROWS == 0 and hkv % RHEADS == 0 and hkv % ZHEADS == 0
  assert (d, d_ff) == (512, 1792)

  row2 = (nb, d)
  b1_shape = (d_ff // 128, 128)
  b2_shape = (d // 128, 128)
  inputs = (A_x.reshape(row2), A_k_cache, A_v_cache, A_wq, A_wo, B_w1,
            B_b1.reshape(b1_shape), B_w2, B_b2.reshape(b2_shape),
            grad_out.reshape(row2))
  out_shapes = (row2, row2, A_k_cache.shape, A_v_cache.shape, A_wq.shape,
                A_wo.shape, B_w1.shape, b1_shape, B_w2.shape, b2_shape)

  def act(n):
    return pltpu.VMEM((N_LAYERS * ROWS, n), F32)

  weights = [pltpu.VMEM(w.shape, BF16) for w in (A_wq, A_wo, B_w1, B_w2)]
  n_rows = N_LAYERS * hkv * ROWS
  scratch = [
      *[pltpu.VMEM(s, BF16) for s in (row2, row2, b1_shape, b2_shape)] * 2,
      *[pltpu.VMEM((nb, hkv, win, dh), BF16)] * 2,
      *weights, *weights,
      pltpu.VMEM((ZHEADS, ZROWS, dh), BF16),
      act(d), act(128), act(d), act(128), act(d_ff), act(d_ff), act(d_ff),
      act(d), act(d), act(HQ * DH), act(HQ * DH),
      *[pltpu.VMEM((n_rows, DH), F32)] * 2,
      pltpu.VMEM((ROWS, d_ff), F32),
      *[pltpu.VMEM((n_rows, win), F32)] * 2,
      pltpu.VMEM((2, nb * hkv, n_rows, DH), BF16),
      pltpu.SemaphoreType.DMA((6,)),
      pltpu.SemaphoreType.DMA((2,)),
      pltpu.SemaphoreType.DMA((6,)),
      pltpu.SemaphoreType.DMA((4,)),
  ]

  outs = pl.pallas_call(
      _kernel,
      out_shape=[jax.ShapeDtypeStruct(s, BF16) for s in out_shapes],
      in_specs=[pl.BlockSpec(memory_space=pltpu.HBM)] * len(inputs),
      out_specs=[pl.BlockSpec(memory_space=pltpu.HBM)] * len(out_shapes),
      scratch_shapes=scratch,
      compiler_params=pltpu.CompilerParams(
          vmem_limit_bytes=100 * 1024 * 1024, disable_bounds_checks=NOBC),
  )(*inputs)
  out, dx, dk, dv, dwq, dwo, dw1, db1, dw2, db2 = outs
  return (out.reshape(A_x.shape), dx.reshape(A_x.shape), dk, dv, dwq, dwo,
          dw1, db1.reshape(B_b1.shape), dw2, db2.reshape(B_b2.shape))
```

```python
import math

import jax
import jax.numpy as jnp
from jax import lax
import jax.experimental.pallas as pl
import jax.experimental.pallas.tpu as pltpu

HQ = 32
DH = 128
EPS = 1e-5
GELU_C = math.sqrt(2.0 / math.pi)
GELU_A = 0.044715
N_LAYERS = 2
ROWS = 8

DMA_HEADS = 4
WIN_ROWS = 32
ZERO_ROWS = 112
W_RUNS = 4
KCHUNK = 512
FCHUNK = 256

PUMP_START = 32
PUMP_ATTN = 12
PUMP_MLP = 3
PUMP_DW = 6
PUMP_CACHE = 20

F32 = jnp.float32
BF16 = jnp.bfloat16


def _nn(a, b):
  return lax.dot_general(a, b, (((1,), (0,)), ((), ())),
                         preferred_element_type=F32)


def _nt(a, b):
  return lax.dot_general(a, b, (((1,), (1,)), ((), ())),
                         preferred_element_type=F32)


def _row_iota(shape):
  return lax.broadcasted_iota(jnp.int32, shape, 0)


def _by_batch(v0, v1):
  return jnp.where(_row_iota(v0.shape) % 2 == 0, v0, v1)


def _layernorm(x):
  xc = x - jnp.mean(x, axis=-1, keepdims=True)
  var = jnp.mean(xc * xc, axis=-1, keepdims=True)
  rstd = 1.0 / jnp.sqrt(var + EPS)
  return xc * rstd, rstd


def _layernorm_bwd(dn, n, rstd):
  return rstd * (dn - jnp.mean(dn, axis=-1, keepdims=True)
                 - n * jnp.mean(dn * n, axis=-1, keepdims=True))


def _gelu_tanh(h):
  return jnp.tanh(GELU_C * (h + GELU_A * h * h * h))


def _sum_head_rows(v):
  v = v + pltpu.roll(v, 4, 0)
  return v + pltpu.roll(v, 2, 0)


def _chunk(i, size):
  return pl.ds(pl.multiple_of(i * size, size), size)


def _loop(lo, hi, body):
  lax.fori_loop(lo, hi, lambda i, c: (body(i), c)[1], 0)


def _wait_total(ref, sem):
  pltpu.make_async_copy(ref, ref, sem).wait()


def _kernel(x_hbm, k_hbm, v_hbm, wq_hbm, wo_hbm, w1_hbm, b1_hbm, w2_hbm,
            b2_hbm, go_hbm,
            out_hbm, dx_hbm, dk_hbm, dv_hbm, dwq_hbm, dwo_hbm, dw1_hbm,
            db1_hbm, dw2_hbm, db2_hbm,
            xs, gos, b1s, b2s, outs, dxs, db1s, db2s,
            kbuf, vbuf, wq, wo, w1, w2, dwq, dwo, dw1, dw2, zbuf,
            na_s, ra_s, nb_s, rb_s, h_s, g_s, dh_s, da_s, dy_s,
            oe_s, dqe_s, q_s, do_s, b1_s, p_s, ds_s, sel_s,
            rsem, zsem, wsem, ssem):
  nb, hkv, seq, _ = k_hbm.shape
  win = kbuf.shape[2]
  zero_rows = seq - win
  rep = HQ // hkv
  gw = rep * DH
  d_ff = w1.shape[1]
  scale = DH ** -0.5
  n_kchunk = win // KCHUNK
  n_fchunk = d_ff // FCHUNK
  head_groups = hkv // DMA_HEADS

  def cache_piece(i, n_chunks, rows):
    grp, c = i // n_chunks, i % n_chunks
    return (grp // head_groups,
            pl.ds(grp % head_groups * DMA_HEADS, DMA_HEADS), c * rows)

  win_chunks = win // WIN_ROWS

  def move_window(to_vmem, sem):
    def step(i):
      b, heads, r = cache_piece(i, win_chunks, WIN_ROWS)
      for q, (hbm, buf) in enumerate(
          ((k_hbm, kbuf), (v_hbm, vbuf)) if to_vmem else
          ((dk_hbm, kbuf), (dv_hbm, vbuf))):
        far = hbm.at[b, heads, pl.ds(zero_rows + r, WIN_ROWS), :]
        near = buf.at[b, heads, pl.ds(r, WIN_ROWS), :]
        src, dst = (far, near) if to_vmem else (near, far)
        pltpu.make_async_copy(src, dst, sem.at[q]).start(priority=q)

    _loop(0, nb * head_groups * win_chunks, step)

  move_window(True, rsem)

  def piece(src, dst, idx, sem, queue):
    pltpu.make_async_copy(src.at[idx], dst.at[idx], sem).start(priority=queue)

  def read_attn_weights(i):
    piece(wq_hbm, wq, (slice(None), pl.ds(i // hkv * 8, 8),
                       pl.ds(i % hkv * gw, gw)), rsem.at[2], 0)
    piece(wo_hbm, wo, (slice(None), pl.ds(i * 8, 8)), rsem.at[3], 1)

  assert wq.shape[1] * hkv == wo.shape[1]
  _loop(0, wo.shape[1] // 8, read_attn_weights)

  def read_mlp_weights(i):
    piece(w1_hbm, w1, (pl.ds(i // 2 * 16, 16),
                       pl.ds(i % 2 * (d_ff // 2), d_ff // 2)), rsem.at[4], 0)

    @pl.when(i < d_ff // 32)
    def _():
      piece(w2_hbm, w2, pl.ds(i * 32, 32), rsem.at[5], 1)

  assert w1.shape[0] // 8 >= d_ff // 32
  _loop(0, w1.shape[0] // 8, read_mlp_weights)

  small_in = [pltpu.make_async_copy(s, d, ssem.at[i]) for i, (s, d) in
              enumerate(((x_hbm, xs), (go_hbm, gos), (b1_hbm, b1s),
                         (b2_hbm, b2s)))]
  for cp in small_in:
    cp.start()

  zbuf[...] = jnp.zeros(zbuf.shape, BF16)
  z_chunks = zero_rows // ZERO_ROWS
  z_total = nb * head_groups * z_chunks

  def zero_step(i):
    b, heads, r = cache_piece(i, z_chunks, ZERO_ROWS)
    for q, dst in enumerate((dk_hbm, dv_hbm)):
      pltpu.make_async_copy(zbuf, dst.at[b, heads, pl.ds(r, ZERO_ROWS), :],
                            zsem.at[q]).start(priority=q)

  def pump(done, n):
    _loop(done, done + n, zero_step)
    return done + n

  assert (PUMP_START + 2 * N_LAYERS * (hkv * PUMP_ATTN + n_fchunk * PUMP_MLP)
          + (hkv + n_fchunk) * PUMP_DW + 2 * n_kchunk * PUMP_CACHE) <= z_total
  zi = pump(jnp.int32(0), PUMP_START)

  for cp in small_in:
    cp.wait()
  for i, buf in enumerate((kbuf, vbuf, wq, wo, w1, w2)):
    _wait_total(buf, rsem.at[i])

  def wq_of(g):
    return wq[:, :, _chunk(g, gw)].reshape(wq.shape[0] * wq.shape[1], gw)

  def wo_of(g):
    per_run = wo.shape[1] // gw
    return wo[g // per_run, _chunk(g % per_run, gw), :]

  def replicate(ref):
    v = ref[...].astype(F32)
    shape = (ROWS, v.shape[1])
    return _by_batch(jnp.broadcast_to(v[0:1], shape),
                     jnp.broadcast_to(v[1:2], shape))

  def bias_rows(ref):
    v = ref[...].astype(F32)
    return jnp.concatenate(
        [jnp.broadcast_to(v[i:i + 1], (ROWS, 128)) for i in range(v.shape[0])],
        axis=1)

  b1_s[...] = bias_rows(b1s)
  b2 = bias_rows(b2s)
  head_of_row = _row_iota((ROWS, DH)) // 2

  def gather_heads(v):
    t = v[:, 0:DH]
    for r in range(1, rep):
      t = jnp.where(head_of_row == r, v[:, r * DH:(r + 1) * DH], t)
    return t

  def scatter_heads(t):
    return jnp.concatenate(
        [jnp.where(head_of_row == r, t, 0.0) for r in range(rep)], axis=1)

  def first_copy(v):
    return jnp.where(_row_iota(v.shape) < nb, v, 0.0)

  def layer_fwd(l, carry):
    x, zi = carry
    rows = _chunk(l, ROWS)
    n, rstd = _layernorm(x)
    na_s[rows, :] = n
    ra_s[rows, :] = jnp.broadcast_to(rstd, (ROWS, 128))
    n = n.astype(BF16)

    def group(g, carry):
      acc, zi = carry
      zi = pump(zi, PUMP_ATTN)
      cols = _chunk(g, gw)
      grows = _chunk(l * hkv + g, ROWS)
      q = gather_heads(_nn(n, wq_of(g)))
      q_s[grows, :] = q
      q = q.astype(BF16)
      s = _by_batch(_nt(q, kbuf[0, g]), _nt(q, kbuf[1, g])) * scale
      e = jnp.exp(s - jnp.max(s, axis=-1, keepdims=True))
      p = e / jnp.sum(e, axis=-1, keepdims=True)
      p_s[grows, :] = p
      p = p.astype(BF16)
      oe = scatter_heads(_by_batch(_nn(p, vbuf[0, g]), _nn(p, vbuf[1, g])))
      oe_s[rows, cols] = oe
      return acc + _nn(oe.astype(BF16), wo_of(g)), zi

    acc, zi = lax.fori_loop(0, hkv, group, (jnp.zeros_like(x), zi))
    x = x + _sum_head_rows(acc)

    n2, rstd = _layernorm(x)
    nb_s[rows, :] = n2
    rb_s[rows, :] = jnp.broadcast_to(rstd, (ROWS, 128))
    n2 = n2.astype(BF16)

    def hidden(j, carry):
      acc, zi = carry
      zi = pump(zi, PUMP_MLP)
      cols = _chunk(j, FCHUNK)
      h = _nn(n2, w1[:, cols]) + b1_s[:, cols]
      h_s[rows, cols] = h
      act = 0.5 * h * (1.0 + _gelu_tanh(h))
      g_s[rows, cols] = act
      return acc + _nn(act.astype(BF16), w2[cols, :]), zi

    acc, zi = lax.fori_loop(0, n_fchunk, hidden, (b2, zi))
    return x + acc, zi

  x, zi = lax.fori_loop(0, N_LAYERS, layer_fwd, (replicate(xs), zi))
  outs[...] = x[0:nb].astype(BF16)

  def layer_bwd(i, carry):
    dx, zi = carry
    l = N_LAYERS - 1 - i
    rows = _chunk(l, ROWS)
    dy_s[rows, :] = first_copy(dx)
    dy = dx.astype(BF16)

    def hidden(j, carry):
      acc, zi = carry
      zi = pump(zi, PUMP_MLP)
      cols = _chunk(j, FCHUNK)
      h = h_s[rows, cols]
      t = _gelu_tanh(h)
      dgelu = 0.5 * (1.0 + t) + (0.5 * GELU_C) * h * (1.0 - t * t) * (
          1.0 + (3.0 * GELU_A) * h * h)
      dh = _nt(dy, w2[cols, :]) * dgelu
      dh_s[rows, cols] = first_copy(dh)
      return acc + _nt(dh.astype(BF16), w1[:, cols]), zi

    dn, zi = lax.fori_loop(0, n_fchunk, hidden, (jnp.zeros_like(dx), zi))
    dx = dx + _layernorm_bwd(dn, nb_s[rows, :], rb_s[rows, 0:1])
    da_s[rows, :] = dx
    da = dx.astype(BF16)

    def group(g, carry):
      acc, zi = carry
      zi = pump(zi, PUMP_ATTN)
      cols = _chunk(g, gw)
      grows = _chunk(l * hkv + g, ROWS)
      do = gather_heads(_nt(da, wo_of(g)))
      do_s[grows, :] = do
      do = do.astype(BF16)
      dp = _by_batch(_nt(do, vbuf[0, g]), _nt(do, vbuf[1, g]))
      p = p_s[grows, :]
      ds = p * (dp - jnp.sum(p * dp, axis=-1, keepdims=True)) * scale
      ds_s[grows, :] = ds
      ds = ds.astype(BF16)
      dqe = scatter_heads(_by_batch(_nn(ds, kbuf[0, g]), _nn(ds, kbuf[1, g])))
      dqe_s[rows, cols] = dqe
      return acc + _nt(dqe.astype(BF16), wq_of(g)), zi

    dn, zi = lax.fori_loop(0, hkv, group, (jnp.zeros_like(dx), zi))
    dx = dx + _layernorm_bwd(_sum_head_rows(dn), na_s[rows, :],
                             ra_s[rows, 0:1])
    return dx, zi

  dx, zi = lax.fori_loop(0, N_LAYERS, layer_bwd, (replicate(gos), zi))
  dxs[...] = dx[0:nb].astype(BF16)

  def weight_grads(n, size, up_act, up_grad, up, down_act, down_grad, down, zi):
    a = up_act[...].T.astype(BF16)
    dg = down_grad[...].astype(BF16)
    per_run = down.shape[1] // size

    def step(j, zi):
      zi = pump(zi, PUMP_DW)
      cols = _chunk(j, size)
      du = _nn(a, up_grad[:, cols].astype(BF16)).astype(BF16)
      up[:, :, cols] = du.reshape(up.shape[0], up.shape[1], size)
      dd = _nn(down_act[:, cols].T.astype(BF16), dg).astype(BF16)
      down[j // per_run, _chunk(j % per_run, size), :] = dd
      return zi

    return lax.fori_loop(0, n, step, zi)

  zi = weight_grads(hkv, gw, na_s, dqe_s, dwq, oe_s, da_s, dwo, zi)
  zi = weight_grads(n_fchunk, FCHUNK, nb_s, dh_s, dw1, g_s, dy_s, dw2, zi)
  for dst, grad in ((db1s, dh_s), (db2s, dy_s)):
    tot = jnp.sum(grad[...], axis=0, keepdims=True)
    dst[...] = jnp.concatenate(
        [tot[:, i * 128:(i + 1) * 128] for i in range(dst.shape[0])],
        axis=0).astype(BF16)

  small_out = [pltpu.make_async_copy(s, d, ssem.at[i]) for i, (s, d) in
               enumerate(((outs, out_hbm), (dxs, dx_hbm), (db1s, db1_hbm),
                          (db2s, db2_hbm)))]
  for cp in small_out:
    cp.start()

  for t, (up, up_hbm, down, down_hbm, width) in enumerate(
      ((dwq, dwq_hbm, dwo, dwo_hbm, 1024), (dw1, dw1_hbm, dw2, dw2_hbm, 896))):
    per_band = up.shape[2] // width
    n_steps = up.shape[1] // 16 * per_band
    down_rows = down.shape[1] // n_steps
    assert down_rows * n_steps == down.shape[1] and down_rows % 16 == 0

    def write_weights(i):
      piece(up, up_hbm, (slice(None), pl.ds(i // per_band * 16, 16),
                         pl.ds(i % per_band * width, width)),
            wsem.at[2 + 2 * t], 0)
      piece(down, down_hbm, (slice(None), pl.ds(i * down_rows, down_rows)),
            wsem.at[3 + 2 * t], 1)

    _loop(0, n_steps, write_weights)

  row = _row_iota(q_s.shape)
  owner = (row % 2) * hkv + (row // ROWS) % hkv

  def select_step(j):
    for t, src in enumerate((q_s, do_s)):
      sel_s[t, j] = jnp.where(owner == j, src[...], 0.0).astype(BF16)

  _loop(0, nb * hkv, select_step)

  def cache_step(c, zi):
    keys = _chunk(c, KCHUNK)
    for t, (src, dst) in enumerate(((ds_s, kbuf), (p_s, vbuf))):
      zi = pump(zi, PUMP_CACHE)
      at = src[:, keys].T.astype(BF16)

      def head_step(j):
        dst[j // hkv, j % hkv, keys, :] = _nn(at, sel_s[t, j]).astype(BF16)

      _loop(0, nb * hkv, head_step)
    return zi

  zi = lax.fori_loop(0, n_kchunk, cache_step, zi)

  _loop(zi, z_total, zero_step)
  move_window(False, wsem)

  for cp in small_out:
    cp.wait()
  for i, dst in enumerate((dwq_hbm, dwo_hbm, dw1_hbm, dw2_hbm)):
    _wait_total(dst, wsem.at[2 + i])
  for q, dst in enumerate((dk_hbm, dv_hbm)):
    _wait_total(dst.at[:, :, pl.ds(0, zero_rows), :], zsem.at[q])
    _wait_total(dst.at[:, :, pl.ds(zero_rows, win), :], wsem.at[q])


@jax.jit
def pallas_interleave_layers__sliding_block_cached__dense_activation_gelu__decode_kernel(
    A_x: jax.Array,
    A_k_cache: jax.Array,
    A_v_cache: jax.Array,
    A_wq: jax.Array,
    A_wo: jax.Array,
    B_x: jax.Array,
    B_w1: jax.Array,
    B_b1: jax.Array,
    B_w2: jax.Array,
    B_b2: jax.Array,
    grad_out: jax.Array,
):
  del B_x
  nb, sq, d = A_x.shape
  _, hkv, seq, dh = A_k_cache.shape
  d_ff = B_w1.shape[1]
  win = min(4096, max(256, seq // 4))
  assert (nb, sq, dh, d, d_ff) == (2, 1, DH, 512, 1792) and HQ == 4 * hkv
  assert win % KCHUNK == 0 and win % WIN_ROWS == 0
  assert (seq - win) % ZERO_ROWS == 0 and hkv % DMA_HEADS == 0

  def runs(rows, cols, n):
    return (n, rows // n, cols)

  row2 = (nb, d)
  b1_shape = (d_ff // 128, 128)
  b2_shape = (d // 128, 128)
  dw_shapes = (runs(d, HQ * DH, W_RUNS), runs(HQ * DH, d, W_RUNS),
               runs(d, d_ff, W_RUNS), runs(d_ff, d, d_ff // FCHUNK))
  inputs = (A_x.reshape(row2), A_k_cache, A_v_cache,
            A_wq.reshape(dw_shapes[0]), A_wo.reshape(dw_shapes[1]), B_w1,
            B_b1.reshape(b1_shape), B_w2, B_b2.reshape(b2_shape),
            grad_out.reshape(row2))
  out_shapes = (row2, row2, A_k_cache.shape, A_v_cache.shape, dw_shapes[0],
                dw_shapes[1], dw_shapes[2], b1_shape, dw_shapes[3], b2_shape)

  def act(n):
    return pltpu.VMEM((N_LAYERS * ROWS, n), F32)

  n_rows = N_LAYERS * hkv * ROWS
  scratch = [
      *[pltpu.VMEM(s, BF16) for s in (row2, row2, b1_shape, b2_shape)] * 2,
      *[pltpu.VMEM((nb, hkv, win, dh), BF16)] * 2,
      *[pltpu.VMEM(s, BF16) for s in (*dw_shapes[:2], B_w1.shape, B_w2.shape)],
      *[pltpu.VMEM(s, BF16) for s in dw_shapes],
      pltpu.VMEM((DMA_HEADS, ZERO_ROWS, dh), BF16),
      act(d), act(128), act(d), act(128), act(d_ff), act(d_ff), act(d_ff),
      act(d), act(d), act(HQ * DH), act(HQ * DH),
      *[pltpu.VMEM((n_rows, DH), F32)] * 2,
      pltpu.VMEM((ROWS, d_ff), F32),
      *[pltpu.VMEM((n_rows, win), F32)] * 2,
      pltpu.VMEM((2, nb * hkv, n_rows, DH), BF16),
      pltpu.SemaphoreType.DMA((6,)),
      pltpu.SemaphoreType.DMA((2,)),
      pltpu.SemaphoreType.DMA((6,)),
      pltpu.SemaphoreType.DMA((4,)),
  ]

  outs = pl.pallas_call(
      _kernel,
      out_shape=[jax.ShapeDtypeStruct(s, BF16) for s in out_shapes],
      in_specs=[pl.BlockSpec(memory_space=pltpu.HBM)] * len(inputs),
      out_specs=[pl.BlockSpec(memory_space=pltpu.HBM)] * len(out_shapes),
      scratch_shapes=scratch,
      compiler_params=pltpu.CompilerParams(
          vmem_limit_bytes=100 * 1024 * 1024),
  )(*inputs)
  like = (A_x, A_x, A_k_cache, A_v_cache, A_wq, A_wo, B_w1, B_b1, B_w2, B_b2)
  return tuple(o.reshape(a.shape) for o, a in zip(outs, like))
```
